```python
import jax
import jax.numpy as jnp

def _softmax(x, axis=-1):
    return jax.nn.softmax(x, axis=axis)
def _gelu(x):
    return jax.nn.gelu(x, approximate=True)
def _silu(x):
    return jax.nn.silu(x)
def _sigmoid(x):
    return jax.nn.sigmoid(x)
def _layernorm(x, axis=-1, eps=1e-5):
    m = jnp.mean(x, axis=axis, keepdims=True)
    v = jnp.var(x, axis=axis, keepdims=True)
    return (x - m) / jnp.sqrt(v + eps)
def _scatter_add(tgt, idx, src, axis=0):
    return tgt.at[idx].add(src)
def _segment_sum(src, seg, n):
    return jax.ops.segment_sum(src, seg, n)
class _Rng:
    def __init__(self, key):
        self._k = key
    def _next(self):
        self._k, sub = jax.random.split(self._k)
        return sub
    def normal(self, shape):
        return jax.random.normal(self._next(), shape, dtype=jnp.bfloat16)
    def randint(self, lo, hi, shape):
        return jax.random.randint(self._next(), shape, lo, hi, dtype=jnp.int32)
    def uniform(self, shape, lo=0.0, hi=1.0):
        return jax.random.uniform(self._next(), shape, jnp.bfloat16, lo, hi)
    def permutation(self, n):
        return jax.random.permutation(self._next(), n)


kernel_name = 'sequential_preLN__mha_block_cached__moe_arch_mod__decode'

def setup_inputs():
    _rng = _Rng(jax.random.key(int.from_bytes(__import__("os").urandom(4), "little")))
    _w = (lambda a: (lambda t: t.astype(jnp.bfloat16) if jnp.issubdtype(t.dtype, jnp.floating) else t)(jnp.asarray(a)))
    def _A_setup():
        B, Sq, D = 4, 1, 640
        H, Sk, Dh = 32, 8192, 192
        return {
            "x": _w((lambda *s: _rng.normal(s) * 0.05)(B, Sq, D)),
            "k_cache": _w((lambda *s: _rng.normal(s) * 0.05)(B, H, Sk, Dh)),
            "v_cache": _w((lambda *s: _rng.normal(s) * 0.05)(B, H, Sk, Dh)),
            "wq": _w((lambda *s: _rng.normal(s) * 0.05)(D, H * Dh) * (D ** -0.5)),
            "wo": _w((lambda *s: _rng.normal(s) * 0.05)(H * Dh, D) * ((H * Dh) ** -0.5)),
        }
    _A_in = _A_setup()

    def _B_setup():
        B, S, D, F, C = 4, 1, 640, 1536, 1
        return {
            "x": _w((lambda *s: _rng.normal(s) * 0.05)(B, S, D)),
            "w_r": _w((lambda *s: _rng.normal(s) * 0.05)(D)),
            "w_gate": _w((lambda *s: _rng.normal(s) * 0.05)(D, F)),
            "w_up": _w((lambda *s: _rng.normal(s) * 0.05)(D, F)),
            "w_down": _w((lambda *s: _rng.normal(s) * 0.05)(F, D)),
        }
    _B_in = _B_setup()

    return {
        "A_x": _A_in["x"],
        "A_k_cache": _A_in["k_cache"],
        "A_v_cache": _A_in["v_cache"],
        "A_wq": _A_in["wq"],
        "A_wo": _A_in["wo"],
        "B_x": _B_in["x"],
        "B_w_r": _B_in["w_r"],
        "B_w_gate": _B_in["w_gate"],
        "B_w_up": _B_in["w_up"],
        "B_w_down": _B_in["w_down"],
    }

def reference(A_x, A_k_cache, A_v_cache, A_wq, A_wo, B_x, B_w_r, B_w_gate, B_w_up, B_w_down):
    def _A_ref(x, k_cache, v_cache, wq, wo):
        B, Sq, D = x.shape
        H, Dh = 32, 192
        q = (lambda x, *d: x.transpose(*d))((x @ wq).reshape(B, Sq, H, Dh), 0, 2, 1, 3)
        scores = jnp.einsum("bhqd,bhkd->bhqk", q, k_cache) * (Dh ** -0.5)
        p = _softmax(scores, axis=-1)
        o = jnp.einsum("bhqk,bhkd->bhqd", p, v_cache)
        return (lambda x, *d: x.transpose(*d))(o, 0, 2, 1, 3).reshape(B, Sq, H * Dh) @ wo

    def _B_ref(x, w_r, w_gate, w_up, w_down):
        B, S, D = x.shape
        C = 1
        r = x @ w_r
        idx = jnp.argsort(-r, axis=-1)[:, :C]
        idx_e = jnp.repeat(idx.reshape(B, C, 1), D, axis=2)
        x_sel = jnp.take_along_axis(x, idx_e, axis=1)
        g = _silu(x_sel @ w_gate)
        u = x_sel @ w_up
        y = (g * u) @ w_down
        r_sel = _sigmoid(jnp.take_along_axis(r, idx, axis=1))
        y = y * r_sel.reshape(B, C, 1)
        b_off = (jnp.arange(B) * S).reshape(B, 1)
        flat_idx = (idx + b_off).reshape(B * C)
        zero = (x * 0.0).reshape(B * S, D)
        upd = _scatter_add(zero, flat_idx, y.reshape(B * C, D), axis=0)
        return x + upd.reshape(B, S, D)

    x = A_x
    h = x + _A_ref(_layernorm(x, axis=-1), A_k_cache, A_v_cache, A_wq, A_wo)
    h2 = h + _B_ref(_layernorm(h, axis=-1), B_w_r, B_w_gate, B_w_up, B_w_down)
    return h2
```

```python
import jax
import jax.numpy as jnp
from jax import lax
import jax.experimental.pallas as pl
import jax.experimental.pallas.tpu as pltpu

B, D, H, SK, DH, F = 4, 640, 32, 8192, 192, 1536
R = 8
NS = 4
NWD = 4
WD_ROWS = F // NWD
TOTAL = B * H
EPS = 1e-5
SCALE = DH ** -0.5
BF = jnp.bfloat16
F32 = jnp.float32


def _layernorm(x):
    m = jnp.mean(x, axis=-1, keepdims=True)
    xc = x - m
    v = jnp.mean(xc * xc, axis=-1, keepdims=True)
    return xc / jnp.sqrt(v + EPS)


def _kernel(x_hbm, k_hbm, v_hbm, wq_hbm, wo_hbm, wr_hbm, wg_hbm, wu_hbm, wd_hbm,
            out_ref,
            x_v, wr_v, wq_v, wo_v, wg_v, wu_v, wd_v, kbuf, vbuf,
            x8_scr, q_scr, o_scr, acc_scr,
            ksem, vsem, msem, dsem):
    def k_copy(i):
        slot = i % NS
        return pltpu.make_async_copy(k_hbm.at[i % B, i // B], kbuf.at[slot], ksem.at[slot])

    def v_copy(i):
        slot = i % NS
        return pltpu.make_async_copy(v_hbm.at[i % B, i // B], vbuf.at[slot], vsem.at[slot])

    x_copy = pltpu.make_async_copy(x_hbm, x_v, msem.at[0])
    wr_copy = pltpu.make_async_copy(wr_hbm, wr_v, msem.at[1])
    wq_copy = pltpu.make_async_copy(wq_hbm, wq_v, msem.at[2])
    wo_copy = pltpu.make_async_copy(wo_hbm, wo_v, msem.at[3])
    wg_copy = pltpu.make_async_copy(wg_hbm, wg_v, msem.at[4])
    wu_copy = pltpu.make_async_copy(wu_hbm, wu_v, msem.at[5])

    def wd_copy(c):
        rows = pl.ds(c * WD_ROWS, WD_ROWS)
        return pltpu.make_async_copy(wd_hbm.at[rows], wd_v.at[rows], dsem.at[c])

    x_copy.start()
    wq_copy.start()
    wr_copy.start()
    for i in range(NS):
        k_copy(i).start()
        v_copy(i).start()
    wo_copy.start()

    x_copy.wait()
    x8_scr[...] = jnp.zeros((R, D), F32)
    x8_scr[0:B, :] = x_v[...].astype(F32)
    xn = _layernorm(x8_scr[...]).astype(BF)
    o_scr[...] = jnp.zeros((R, DH), F32)
    acc_scr[...] = jnp.zeros((R, D), F32)

    wq_copy.wait()
    q_all = jnp.dot(xn, wq_v[...], preferred_element_type=F32)
    for h in range(H):
        q_scr[h] = q_all[:, h * DH:(h + 1) * DH].astype(BF)

    rows = lax.broadcasted_iota(jnp.int32, (R, DH), 0)

    def body(i, carry):
        slot = i % NS
        b = i % B
        h = i // B
        k_copy(i).wait()
        s = jnp.dot(q_scr[h], kbuf[slot], preferred_element_type=F32)
        m = jnp.max(s, axis=-1, keepdims=True)
        p = jnp.exp((s - m) * SCALE)
        l = jnp.sum(p, axis=-1, keepdims=True)
        pb = p.astype(BF)

        @pl.when(i + NS < TOTAL)
        def _():
            k_copy(i + NS).start()

        v_copy(i).wait()
        o = lax.dot_general(pb, vbuf[slot], (((1,), (1,)), ((), ())),
                            preferred_element_type=F32)

        @pl.when(i + NS < TOTAL)
        def _():
            v_copy(i + NS).start()

        @pl.when(i + NS == TOTAL - 1)
        def _():
            wg_copy.start()
            wu_copy.start()
            for c in range(NWD):
                wd_copy(c).start()

        o_scr[...] = jnp.where(rows == b, o / l, o_scr[...])

        @pl.when(i == B - 1)
        def _():
            wo_copy.wait()

        @pl.when(b == B - 1)
        def _():
            wo_h = wo_v[pl.ds(pl.multiple_of(h * DH, DH), DH), :]
            acc_scr[...] += jnp.dot(o_scr[...].astype(BF), wo_h, preferred_element_type=F32)
        return carry

    lax.fori_loop(0, TOTAL, body, 0)

    hres = x8_scr[...] + acc_scr[...]
    hn = _layernorm(hres)
    hb = hn.astype(BF)
    wr_copy.wait()
    wr = wr_v[...].astype(F32)
    racc = hn[:, 0:128] * wr[0:1, :]
    for j in range(1, D // 128):
        racc = racc + hn[:, j * 128:(j + 1) * 128] * wr[j:j + 1, :]
    gate = jax.nn.sigmoid(jnp.sum(racc, axis=-1, keepdims=True))
    base = hres + hn + hn * 0.0

    wg_copy.wait()
    g = jnp.dot(hb, wg_v[...], preferred_element_type=F32)
    g = g * jax.nn.sigmoid(g)
    wu_copy.wait()
    u = jnp.dot(hb, wu_v[...], preferred_element_type=F32)
    act = (g * u).astype(BF)
    y = None
    for c in range(NWD):
        wd_copy(c).wait()
        part = jnp.dot(act[:, c * WD_ROWS:(c + 1) * WD_ROWS], wd_v[c * WD_ROWS:(c + 1) * WD_ROWS, :],
                       preferred_element_type=F32)
        y = part if y is None else y + part
    res = base + y * gate
    out_ref[...] = res[0:B, :].astype(BF)


@jax.jit
def pallas_sequential_preLN__mha_block_cached__moe_arch_mod__decode_kernel(
    A_x, A_k_cache, A_v_cache, A_wq, A_wo, B_x, B_w_r, B_w_gate, B_w_up, B_w_down,
):
    x2 = A_x.reshape(B, D)
    kt = jnp.swapaxes(A_k_cache, 2, 3)
    vt = jnp.swapaxes(A_v_cache, 2, 3)
    wr2 = B_w_r.reshape(D // 128, 128)
    any_spec = pl.BlockSpec(memory_space=pl.ANY)
    out = pl.pallas_call(
        _kernel,
        out_shape=jax.ShapeDtypeStruct((B, D), BF),
        in_specs=[any_spec] * 9,
        out_specs=pl.BlockSpec(memory_space=pltpu.VMEM),
        scratch_shapes=[
            pltpu.VMEM((B, D), BF),
            pltpu.VMEM((D // 128, 128), BF),
            pltpu.VMEM((D, H * DH), BF),
            pltpu.VMEM((H * DH, D), BF),
            pltpu.VMEM((D, F), BF),
            pltpu.VMEM((D, F), BF),
            pltpu.VMEM((F, D), BF),
            pltpu.VMEM((NS, DH, SK), BF),
            pltpu.VMEM((NS, DH, SK), BF),
            pltpu.VMEM((R, D), F32),
            pltpu.VMEM((H, R, DH), BF),
            pltpu.VMEM((R, DH), F32),
            pltpu.VMEM((R, D), F32),
            pltpu.SemaphoreType.DMA((NS,)),
            pltpu.SemaphoreType.DMA((NS,)),
            pltpu.SemaphoreType.DMA((6,)),
            pltpu.SemaphoreType.DMA((NWD,)),
        ],
        compiler_params=pltpu.CompilerParams(vmem_limit_bytes=100 * 1024 * 1024),
    )(x2, kt, vt, A_wq, A_wo, wr2, B_w_gate, B_w_up, B_w_down)
    return out.reshape(B, 1, D)
```

```python
import jax
import jax.numpy as jnp
from jax import lax
import jax.experimental.pallas as pl
import jax.experimental.pallas.tpu as pltpu

B, D, H, SK, DH, F = 4, 640, 32, 8192, 192, 1536
R = 8
NS = 4
NWD = 4
WD_ROWS = F // NWD
TOTAL = B * H
CW = 128
EPS = 1e-5
SCALE = DH ** -0.5
BF = jnp.bfloat16
F32 = jnp.float32


def _layernorm(x):
    m = jnp.mean(x, axis=-1, keepdims=True)
    xc = x - m
    v = jnp.mean(xc * xc, axis=-1, keepdims=True)
    return xc / jnp.sqrt(v + EPS)


def _kernel(x_hbm, k_hbm, v_hbm, wq_hbm, wo_hbm, wr_hbm, wg_hbm, wu_hbm, wd_hbm,
            out_ref,
            x_v, wr_v, wq_v, wo_v, wg_v, wu_v, wd_v, kbuf, vbuf,
            x8_scr, q_scr, o_scr, acc_scr,
            ksem, vsem, msem, dsem):
    def slab_start(src, dst, sem, i):
        slot = i % NS
        b = i % B
        h = i // B

        def issue(c, carry):
            for j in range(2):
                cols = pl.ds(pl.multiple_of((2 * c + j) * CW, CW), CW)
                pltpu.make_async_copy(src.at[b, h, :, cols], dst.at[slot, :, cols],
                                      sem.at[slot]).start(priority=j)
            return carry

        lax.fori_loop(0, SK // (2 * CW), issue, 0)

    def slab_wait(dst, sem, i):
        slot = i % NS
        pltpu.make_async_copy(dst.at[slot], dst.at[slot], sem.at[slot]).wait()

    x_copy = pltpu.make_async_copy(x_hbm, x_v, msem.at[0])
    wr_copy = pltpu.make_async_copy(wr_hbm, wr_v, msem.at[1])
    wq_copy = pltpu.make_async_copy(wq_hbm, wq_v, msem.at[2])
    wo_copy = pltpu.make_async_copy(wo_hbm, wo_v, msem.at[3])
    wg_copy = pltpu.make_async_copy(wg_hbm, wg_v, msem.at[4])
    wu_copy = pltpu.make_async_copy(wu_hbm, wu_v, msem.at[5])

    def wd_copy(c):
        rows = pl.ds(c * WD_ROWS, WD_ROWS)
        return pltpu.make_async_copy(wd_hbm.at[rows], wd_v.at[rows], dsem.at[c])

    x_copy.start()
    wq_copy.start()
    wr_copy.start()
    for i in range(NS):
        slab_start(k_hbm, kbuf, ksem, i)
        slab_start(v_hbm, vbuf, vsem, i)
    wo_copy.start()

    x_copy.wait()
    x8_scr[...] = jnp.zeros((R, D), F32)
    x8_scr[0:B, :] = x_v[...].astype(F32)
    xn = _layernorm(x8_scr[...]).astype(BF)
    o_scr[...] = jnp.zeros((R, DH), F32)
    acc_scr[...] = jnp.zeros((R, D), F32)

    wq_copy.wait()
    q_all = jnp.dot(xn, wq_v[...], preferred_element_type=F32)
    for h in range(H):
        q_scr[h] = q_all[:, h * DH:(h + 1) * DH].astype(BF)

    rows = lax.broadcasted_iota(jnp.int32, (R, DH), 0)

    def body(i, carry):
        slot = i % NS
        b = i % B
        h = i // B
        slab_wait(kbuf, ksem, i)
        s = jnp.dot(q_scr[h], kbuf[slot], preferred_element_type=F32)
        m = jnp.max(s, axis=-1, keepdims=True)
        p = jnp.exp((s - m) * SCALE)
        l = jnp.sum(p, axis=-1, keepdims=True)
        pb = p.astype(BF)

        @pl.when(i + NS < TOTAL)
        def _():
            slab_start(k_hbm, kbuf, ksem, i + NS)

        slab_wait(vbuf, vsem, i)
        o = lax.dot_general(pb, vbuf[slot], (((1,), (1,)), ((), ())),
                            preferred_element_type=F32)

        @pl.when(i + NS < TOTAL)
        def _():
            slab_start(v_hbm, vbuf, vsem, i + NS)

        @pl.when(i + NS == TOTAL - 1)
        def _():
            wg_copy.start()
            wu_copy.start()
            for c in range(NWD):
                wd_copy(c).start()

        o_scr[...] = jnp.where(rows == b, o / l, o_scr[...])

        @pl.when(i == B - 1)
        def _():
            wo_copy.wait()

        @pl.when(b == B - 1)
        def _():
            wo_h = wo_v[pl.ds(pl.multiple_of(h * DH, DH), DH), :]
            acc_scr[...] += jnp.dot(o_scr[...].astype(BF), wo_h, preferred_element_type=F32)
        return carry

    lax.fori_loop(0, TOTAL, body, 0)

    hres = x8_scr[...] + acc_scr[...]
    hn = _layernorm(hres)
    hb = hn.astype(BF)
    wr_copy.wait()
    wr = wr_v[...].astype(F32)
    racc = hn[:, 0:128] * wr[0:1, :]
    for j in range(1, D // 128):
        racc = racc + hn[:, j * 128:(j + 1) * 128] * wr[j:j + 1, :]
    gate = jax.nn.sigmoid(jnp.sum(racc, axis=-1, keepdims=True))
    base = hres + hn + hn * 0.0

    wg_copy.wait()
    g = jnp.dot(hb, wg_v[...], preferred_element_type=F32)
    g = g * jax.nn.sigmoid(g)
    wu_copy.wait()
    u = jnp.dot(hb, wu_v[...], preferred_element_type=F32)
    act = (g * u).astype(BF)
    y = None
    for c in range(NWD):
        wd_copy(c).wait()
        part = jnp.dot(act[:, c * WD_ROWS:(c + 1) * WD_ROWS], wd_v[c * WD_ROWS:(c + 1) * WD_ROWS, :],
                       preferred_element_type=F32)
        y = part if y is None else y + part
    res = base + y * gate
    out_ref[...] = res[0:B, :].astype(BF)


@jax.jit
def pallas_sequential_preLN__mha_block_cached__moe_arch_mod__decode_kernel(
    A_x, A_k_cache, A_v_cache, A_wq, A_wo, B_x, B_w_r, B_w_gate, B_w_up, B_w_down,
):
    x2 = A_x.reshape(B, D)
    kt = jnp.swapaxes(A_k_cache, 2, 3)
    vt = jnp.swapaxes(A_v_cache, 2, 3)
    wr2 = B_w_r.reshape(D // 128, 128)
    any_spec = pl.BlockSpec(memory_space=pl.ANY)
    out = pl.pallas_call(
        _kernel,
        out_shape=jax.ShapeDtypeStruct((B, D), BF),
        in_specs=[any_spec] * 9,
        out_specs=pl.BlockSpec(memory_space=pltpu.VMEM),
        scratch_shapes=[
            pltpu.VMEM((B, D), BF),
            pltpu.VMEM((D // 128, 128), BF),
            pltpu.VMEM((D, H * DH), BF),
            pltpu.VMEM((H * DH, D), BF),
            pltpu.VMEM((D, F), BF),
            pltpu.VMEM((D, F), BF),
            pltpu.VMEM((F, D), BF),
            pltpu.VMEM((NS, DH, SK), BF),
            pltpu.VMEM((NS, DH, SK), BF),
            pltpu.VMEM((R, D), F32),
            pltpu.VMEM((H, R, DH), BF),
            pltpu.VMEM((R, DH), F32),
            pltpu.VMEM((R, D), F32),
            pltpu.SemaphoreType.DMA((NS,)),
            pltpu.SemaphoreType.DMA((NS,)),
            pltpu.SemaphoreType.DMA((6,)),
            pltpu.SemaphoreType.DMA((NWD,)),
        ],
        compiler_params=pltpu.CompilerParams(vmem_limit_bytes=100 * 1024 * 1024),
    )(x2, kt, vt, A_wq, A_wo, wr2, B_w_gate, B_w_up, B_w_down)
    return out.reshape(B, 1, D)
```

```python
import jax
import jax.numpy as jnp
from jax import lax
import jax.experimental.pallas as pl
import jax.experimental.pallas.tpu as pltpu

B, D, H, SK, DH, F = 4, 640, 32, 8192, 192, 1536
R = 8
NS = 2
CW = 128
TOTAL = B * H
WQ_ROWS = 8
WO_ROWS = 64
WG_ROWS = 32
WD_ROWS = 64
NWD = 4
WD_GROUP = F // NWD
EPS = 1e-5
SCALE = DH ** -0.5
BF = jnp.bfloat16
F32 = jnp.float32


def _layernorm(x):
    m = jnp.mean(x, axis=-1, keepdims=True)
    xc = x - m
    v = jnp.mean(xc * xc, axis=-1, keepdims=True)
    return xc / jnp.sqrt(v + EPS)


def _kernel(x_hbm, k_hbm, v_hbm, wq_hbm, wo_hbm, wr_hbm, wg_hbm, wu_hbm, wd_hbm,
            out_ref,
            x_v, wr_v, wq_v, wo_v, wg_v, wu_v, wd_v, kbuf, vbuf,
            x8_scr, q_scr, acc_scr,
            ksem, vsem, msem, dsem):
    def slab_start(src, dst, sem, i):
        slot = i % NS
        b = i // H
        h = i % H

        def issue(c, carry):
            for j in range(2):
                cols = pl.ds(pl.multiple_of((2 * c + j) * CW, CW), CW)
                pltpu.make_async_copy(src.at[b, h, :, cols], dst.at[slot, :, cols],
                                      sem.at[slot]).start(priority=j)
            return carry

        lax.fori_loop(0, SK // (2 * CW), issue, 0)

    def rows_start(src, dst, sem, row0, nrows, step):
        def issue(c, carry):
            for j in range(2):
                rows = pl.ds(pl.multiple_of(row0 + (2 * c + j) * step, step), step)
                pltpu.make_async_copy(src.at[rows], dst.at[rows], sem).start(priority=j)
            return carry

        lax.fori_loop(0, nrows // (2 * step), issue, 0)

    def wait_all(dst, sem):
        pltpu.make_async_copy(dst, dst, sem).wait()

    x_copy = pltpu.make_async_copy(x_hbm, x_v, msem.at[0])
    wr_copy = pltpu.make_async_copy(wr_hbm, wr_v, msem.at[1])

    x_copy.start()
    wr_copy.start(priority=1)
    rows_start(wq_hbm, wq_v, msem.at[2], 0, D, WQ_ROWS)
    slab_start(k_hbm, kbuf, ksem, 0)
    slab_start(v_hbm, vbuf, vsem, 0)

    x_copy.wait()
    x8_scr[...] = jnp.zeros((R, D), F32)
    x8_scr[0:B, :] = x_v[...].astype(F32)
    xn = _layernorm(x8_scr[...]).astype(BF)
    acc_scr[...] = jnp.zeros((R, D), F32)

    wait_all(wq_v, msem.at[2])
    q_all = jnp.dot(xn, wq_v[...], preferred_element_type=F32)
    for h in range(H):
        q_scr[h] = q_all[:, h * DH:(h + 1) * DH].astype(BF)

    rows = lax.broadcasted_iota(jnp.int32, (R, DH), 0)

    def body(i, carry):
        slot = i % NS
        b = i // H
        h = i % H
        wait_all(kbuf.at[slot], ksem.at[slot])

        @pl.when(i == 0)
        def _():
            rows_start(wo_hbm, wo_v, msem.at[3], 0, H * DH, WO_ROWS)

        @pl.when(i + 1 < TOTAL)
        def _():
            slab_start(k_hbm, kbuf, ksem, i + 1)

        @pl.when(i + 1 == TOTAL)
        def _():
            rows_start(wg_hbm, wg_v, msem.at[4], 0, D, WG_ROWS)
            rows_start(wu_hbm, wu_v, msem.at[5], 0, D, WG_ROWS)
            for c in range(NWD):
                rows_start(wd_hbm, wd_v, dsem.at[c], c * WD_GROUP, WD_GROUP, WD_ROWS)

        s = jnp.dot(q_scr[h], kbuf[slot], preferred_element_type=F32)
        m = jnp.max(s, axis=-1, keepdims=True)
        p = jnp.exp((s - m) * SCALE)
        l = jnp.sum(p, axis=-1, keepdims=True)
        pb = p.astype(BF)

        wait_all(vbuf.at[slot], vsem.at[slot])

        @pl.when(i + 1 < TOTAL)
        def _():
            slab_start(v_hbm, vbuf, vsem, i + 1)

        o = lax.dot_general(pb, vbuf[slot], (((1,), (1,)), ((), ())),
                            preferred_element_type=F32)

        @pl.when(i == 0)
        def _():
            wait_all(wo_v, msem.at[3])

        ob = jnp.where(rows == b, o / l, 0.0).astype(BF)
        wo_h = wo_v[pl.ds(pl.multiple_of(h * DH, DH), DH), :]
        acc_scr[...] += jnp.dot(ob, wo_h, preferred_element_type=F32)
        return carry

    lax.fori_loop(0, TOTAL, body, 0)

    hres = x8_scr[...] + acc_scr[...]
    hn = _layernorm(hres)
    hb = hn.astype(BF)
    wr_copy.wait()
    wr = wr_v[...].astype(F32)
    racc = hn[:, 0:128] * wr[0:1, :]
    for j in range(1, D // 128):
        racc = racc + hn[:, j * 128:(j + 1) * 128] * wr[j:j + 1, :]
    gate = jax.nn.sigmoid(jnp.sum(racc, axis=-1, keepdims=True))
    base = hres + hn + hn * 0.0

    wait_all(wg_v, msem.at[4])
    g = jnp.dot(hb, wg_v[...], preferred_element_type=F32)
    g = g * jax.nn.sigmoid(g)
    wait_all(wu_v, msem.at[5])
    u = jnp.dot(hb, wu_v[...], preferred_element_type=F32)
    act = (g * u).astype(BF)
    y = None
    for c in range(NWD):
        rows_c = pl.ds(c * WD_GROUP, WD_GROUP)
        wait_all(wd_v.at[rows_c], dsem.at[c])
        part = jnp.dot(act[:, c * WD_GROUP:(c + 1) * WD_GROUP], wd_v[rows_c, :],
                       preferred_element_type=F32)
        y = part if y is None else y + part
    res = base + y * gate
    out_ref[...] = res[0:B, :].astype(BF)


@jax.jit
def pallas_sequential_preLN__mha_block_cached__moe_arch_mod__decode_kernel(
    A_x, A_k_cache, A_v_cache, A_wq, A_wo, B_x, B_w_r, B_w_gate, B_w_up, B_w_down,
):
    x2 = A_x.reshape(B, D)
    kt = jnp.swapaxes(A_k_cache, 2, 3)
    vt = jnp.swapaxes(A_v_cache, 2, 3)
    wr2 = B_w_r.reshape(D // 128, 128)
    any_spec = pl.BlockSpec(memory_space=pl.ANY)
    out = pl.pallas_call(
        _kernel,
        out_shape=jax.ShapeDtypeStruct((B, D), BF),
        in_specs=[any_spec] * 9,
        out_specs=pl.BlockSpec(memory_space=pltpu.VMEM),
        scratch_shapes=[
            pltpu.VMEM((B, D), BF),
            pltpu.VMEM((D // 128, 128), BF),
            pltpu.VMEM((D, H * DH), BF),
            pltpu.VMEM((H * DH, D), BF),
            pltpu.VMEM((D, F), BF),
            pltpu.VMEM((D, F), BF),
            pltpu.VMEM((F, D), BF),
            pltpu.VMEM((NS, DH, SK), BF),
            pltpu.VMEM((NS, DH, SK), BF),
            pltpu.VMEM((R, D), F32),
            pltpu.VMEM((H, R, DH), BF),
            pltpu.VMEM((R, D), F32),
            pltpu.SemaphoreType.DMA((NS,)),
            pltpu.SemaphoreType.DMA((NS,)),
            pltpu.SemaphoreType.DMA((6,)),
            pltpu.SemaphoreType.DMA((NWD,)),
        ],
        compiler_params=pltpu.CompilerParams(vmem_limit_bytes=100 * 1024 * 1024),
    )(x2, kt, vt, A_wq, A_wo, wr2, B_w_gate, B_w_up, B_w_down)
    return out.reshape(B, 1, D)
```

```python
import jax
import jax.numpy as jnp
from jax import lax
import jax.experimental.pallas as pl
import jax.experimental.pallas.tpu as pltpu

B, D, H, SK, DH, F = 4, 640, 32, 8192, 192, 1536
R = 8
HP = 16
UC = 512
NA = DH // 8
NG = B * H // HP
GPB = H // HP
GW = HP * DH
NCH = SK // UC
NU = NG * 2 * NCH
LA = 2
NSLOT = LA + 1
CW = 128
WQ_ROWS = 8
WO_ROWS = 64
WG_ROWS = 32
WD_ROWS = 64
NWD = 4
WD_GROUP = F // NWD
EPS = 1e-5
SCALE = DH ** -0.5
BF = jnp.bfloat16
F32 = jnp.float32


def _layernorm(x):
    m = jnp.mean(x, axis=-1, keepdims=True)
    xc = x - m
    v = jnp.mean(xc * xc, axis=-1, keepdims=True)
    return xc / jnp.sqrt(v + EPS)


def _kernel(x_hbm, k_hbm, v_hbm, wq_hbm, wo_hbm, wr_hbm, wg_hbm, wu_hbm, wd_hbm,
            out_ref,
            x_v, wr_v, wq_v, wo_v, wg_v, wu_v, wd_v, buf,
            x8_scr, qblk_scr, s_scr, p_scr, o_scr, acc_scr,
            usem, msem, dsem):
    def unit_start_from(src, g, ch, slot):
        def issue(j, carry):
            for c in range(UC // CW):
                scol = pl.ds(pl.multiple_of(ch * UC + c * CW, CW), CW)
                pltpu.make_async_copy(src.at[g, :, j, :, scol],
                                      buf.at[slot, :, j, :, pl.ds(c * CW, CW)],
                                      usem.at[slot]).start(priority=c % 2)
            return carry

        lax.fori_loop(0, HP, issue, 0)

    def unit_start(u):
        g = u // (2 * NCH)
        r = u % (2 * NCH)
        ch = r % NCH
        slot = u % NSLOT

        @pl.when(r < NCH)
        def _():
            unit_start_from(k_hbm, g, ch, slot)

        @pl.when(r >= NCH)
        def _():
            unit_start_from(v_hbm, g, ch, slot)

    def rows_start(src, dst, sem, row0, nrows, step):
        def issue(c, carry):
            for j in range(2):
                rows = pl.ds(pl.multiple_of(row0 + (2 * c + j) * step, step), step)
                pltpu.make_async_copy(src.at[rows], dst.at[rows], sem).start(priority=j)
            return carry

        lax.fori_loop(0, nrows // (2 * step), issue, 0)

    def wait_all(dst, sem):
        pltpu.make_async_copy(dst, dst, sem).wait()

    def advance(u):
        slot = u % NSLOT
        wait_all(buf.at[slot], usem.at[slot])

        @pl.when(u == 0)
        def _():
            rows_start(wo_hbm, wo_v, msem.at[3], 0, H * DH, WO_ROWS)

        @pl.when(u + LA < NU)
        def _():
            unit_start(u + LA)

        @pl.when(u + LA == NU)
        def _():
            rows_start(wg_hbm, wg_v, msem.at[4], 0, D, WG_ROWS)
            rows_start(wu_hbm, wu_v, msem.at[5], 0, D, WG_ROWS)
            for c in range(NWD):
                rows_start(wd_hbm, wd_v, dsem.at[c], c * WD_GROUP, WD_GROUP, WD_ROWS)

        return slot

    x_copy = pltpu.make_async_copy(x_hbm, x_v, msem.at[0])
    wr_copy = pltpu.make_async_copy(wr_hbm, wr_v, msem.at[1])

    x_copy.start()
    wr_copy.start(priority=1)
    rows_start(wq_hbm, wq_v, msem.at[2], 0, D, WQ_ROWS)
    for u in range(LA):
        unit_start(u)

    x_copy.wait()
    x8_scr[...] = jnp.zeros((R, D), F32)
    x8_scr[0:B, :] = x_v[...].astype(F32)
    xn = _layernorm(x8_scr[...]).astype(BF)
    acc_scr[...] = jnp.zeros((R, D), F32)

    def head_mask():
        row = lax.broadcasted_iota(jnp.int32, (HP, GW), 0)
        col = lax.broadcasted_iota(jnp.int32, (HP, GW), 1)
        lo = row * DH
        return jnp.logical_and(col >= lo, col < lo + DH)

    wait_all(wq_v, msem.at[2])
    q_all = jnp.dot(xn, wq_v[...], preferred_element_type=F32)
    mask = head_mask()
    for g in range(NG):
        b, hg = g // GPB, g % GPB
        qrow = jnp.broadcast_to(q_all[b:b + 1, hg * GW:(hg + 1) * GW], (HP, GW))
        qblk_scr[g] = jnp.where(mask, qrow, 0.0).astype(BF)

    def group(g, carry):
        u0 = g * (2 * NCH)

        def k_unit(ch, c2):
            slot = advance(u0 + ch)
            kt = buf[slot].reshape(GW, UC)
            col = pl.ds(pl.multiple_of(ch * UC, UC), UC)
            s_scr[:, col] = jnp.dot(qblk_scr[g], kt, preferred_element_type=F32)
            return c2

        lax.fori_loop(0, NCH, k_unit, 0)

        s = s_scr[...]
        m = jnp.max(s, axis=-1, keepdims=True)
        p = jnp.exp((s - m) * SCALE)
        l = jnp.sum(p, axis=-1, keepdims=True)
        p_scr[...] = p.astype(BF)
        o_scr[...] = jnp.zeros((HP, GW), F32)

        def v_unit(ch, c2):
            slot = advance(u0 + NCH + ch)
            vt = buf[slot].reshape(GW, UC)
            col = pl.ds(pl.multiple_of(ch * UC, UC), UC)
            o_scr[...] += lax.dot_general(p_scr[:, col], vt, (((1,), (1,)), ((), ())),
                                          preferred_element_type=F32)
            return c2

        lax.fori_loop(0, NCH, v_unit, 0)

        @pl.when(g == 0)
        def _():
            wait_all(wo_v, msem.at[3])

        ob = jnp.where(head_mask(), o_scr[...] / l, 0.0).astype(BF)
        wo_g = wo_v[pl.ds(pl.multiple_of((g % GPB) * GW, GW), GW), :]
        contrib = jnp.sum(jnp.dot(ob, wo_g, preferred_element_type=F32), axis=0, keepdims=True)
        rows = lax.broadcasted_iota(jnp.int32, (R, D), 0)
        acc_scr[...] += jnp.where(rows == g // GPB, contrib, 0.0)
        return carry

    lax.fori_loop(0, NG, group, 0)

    hres = x8_scr[...] + acc_scr[...]
    hn = _layernorm(hres)
    hb = hn.astype(BF)
    wr_copy.wait()
    wr = wr_v[...].astype(F32)
    racc = hn[:, 0:128] * wr[0:1, :]
    for j in range(1, D // 128):
        racc = racc + hn[:, j * 128:(j + 1) * 128] * wr[j:j + 1, :]
    gate = jax.nn.sigmoid(jnp.sum(racc, axis=-1, keepdims=True))
    base = hres + hn + hn * 0.0

    wait_all(wg_v, msem.at[4])
    g = jnp.dot(hb, wg_v[...], preferred_element_type=F32)
    g = g * jax.nn.sigmoid(g)
    wait_all(wu_v, msem.at[5])
    u = jnp.dot(hb, wu_v[...], preferred_element_type=F32)
    act = (g * u).astype(BF)
    y = None
    for c in range(NWD):
        rows_c = pl.ds(c * WD_GROUP, WD_GROUP)
        wait_all(wd_v.at[rows_c], dsem.at[c])
        part = jnp.dot(act[:, c * WD_GROUP:(c + 1) * WD_GROUP], wd_v[rows_c, :],
                       preferred_element_type=F32)
        y = part if y is None else y + part
    res = base + y * gate
    out_ref[...] = res[0:B, :].astype(BF)


@jax.jit
def pallas_sequential_preLN__mha_block_cached__moe_arch_mod__decode_kernel(
    A_x, A_k_cache, A_v_cache, A_wq, A_wo, B_x, B_w_r, B_w_gate, B_w_up, B_w_down,
):
    x2 = A_x.reshape(B, D)
    kt = jnp.swapaxes(A_k_cache, 2, 3).reshape(NG, NA, HP, 8, SK)
    vt = jnp.swapaxes(A_v_cache, 2, 3).reshape(NG, NA, HP, 8, SK)
    wr2 = B_w_r.reshape(D // 128, 128)
    any_spec = pl.BlockSpec(memory_space=pl.ANY)
    out = pl.pallas_call(
        _kernel,
        out_shape=jax.ShapeDtypeStruct((B, D), BF),
        in_specs=[any_spec] * 9,
        out_specs=pl.BlockSpec(memory_space=pltpu.VMEM),
        scratch_shapes=[
            pltpu.VMEM((B, D), BF),
            pltpu.VMEM((D // 128, 128), BF),
            pltpu.VMEM((D, H * DH), BF),
            pltpu.VMEM((H * DH, D), BF),
            pltpu.VMEM((D, F), BF),
            pltpu.VMEM((D, F), BF),
            pltpu.VMEM((F, D), BF),
            pltpu.VMEM((NSLOT, NA, HP, 8, UC), BF),
            pltpu.VMEM((R, D), F32),
            pltpu.VMEM((NG, HP, GW), BF),
            pltpu.VMEM((HP, SK), F32),
            pltpu.VMEM((HP, SK), BF),
            pltpu.VMEM((HP, GW), F32),
            pltpu.VMEM((R, D), F32),
            pltpu.SemaphoreType.DMA((NSLOT,)),
            pltpu.SemaphoreType.DMA((6,)),
            pltpu.SemaphoreType.DMA((NWD,)),
        ],
        compiler_params=pltpu.CompilerParams(vmem_limit_bytes=100 * 1024 * 1024),
    )(x2, kt, vt, A_wq, A_wo, wr2, B_w_gate, B_w_up, B_w_down)
    return out.reshape(B, 1, D)
```

```python
import jax
import jax.numpy as jnp
from jax import lax
import jax.experimental.pallas as pl
import jax.experimental.pallas.tpu as pltpu

B, D, H, SK, DH, F = 4, 640, 32, 8192, 192, 1536
R = 8
T = 256
NA = 16
UC = 1024
NJ = T // NA
GW = T * 8
HD = H * DH
NRG = HD // GW
NCH = SK // UC
UPB = NRG * NCH
NU = B * 2 * UPB
LA = 2
NSLOT = LA + 1
CW = 128
WQ_ROWS = 8
WO_ROWS = 64
WG_ROWS = 32
WD_ROWS = 64
NWD = 4
WD_GROUP = F // NWD
EPS = 1e-5
SCALE = DH ** -0.5
BF = jnp.bfloat16
F32 = jnp.float32


def _layernorm(x):
    m = jnp.mean(x, axis=-1, keepdims=True)
    xc = x - m
    v = jnp.mean(xc * xc, axis=-1, keepdims=True)
    return xc / jnp.sqrt(v + EPS)


def _kernel(x_hbm, k_hbm, v_hbm, wq_hbm, wo_hbm, wr_hbm, wg_hbm, wu_hbm, wd_hbm,
            out_ref,
            x_v, wr_v, wq_v, wo_v, wg_v, wu_v, wd_v, buf,
            x8_scr, qblk_scr, s_scr, p_scr, l_scr, o_scr, acc_scr,
            usem, msem, dsem):
    def unit_start_from(src, g, ch, slot):
        def issue(j, carry):
            for c in range(UC // CW):
                scol = pl.ds(pl.multiple_of(ch * UC + c * CW, CW), CW)
                pltpu.make_async_copy(src.at[g, :, j, :, scol],
                                      buf.at[slot, :, j, :, pl.ds(c * CW, CW)],
                                      usem.at[slot]).start(priority=c % 2)
            return carry

        lax.fori_loop(0, NJ, issue, 0)

    def unit_start(u):
        b = u // (2 * UPB)
        r = u % (2 * UPB)
        ru = r % UPB
        g = b * NRG + ru // NCH
        ch = ru % NCH
        slot = u % NSLOT

        @pl.when(r < UPB)
        def _():
            unit_start_from(k_hbm, g, ch, slot)

        @pl.when(r >= UPB)
        def _():
            unit_start_from(v_hbm, g, ch, slot)

    def rows_start(src, dst, sem, row0, nrows, step):
        def issue(c, carry):
            for j in range(2):
                rows = pl.ds(pl.multiple_of(row0 + (2 * c + j) * step, step), step)
                pltpu.make_async_copy(src.at[rows], dst.at[rows], sem).start(priority=j)
            return carry

        lax.fori_loop(0, nrows // (2 * step), issue, 0)

    def wait_all(dst, sem):
        pltpu.make_async_copy(dst, dst, sem).wait()

    def advance(u):
        slot = u % NSLOT
        wait_all(buf.at[slot], usem.at[slot])

        @pl.when(u == 0)
        def _():
            rows_start(wo_hbm, wo_v, msem.at[3], 0, H * DH, WO_ROWS)

        @pl.when(u + LA < NU)
        def _():
            unit_start(u + LA)

        @pl.when(u + LA == NU)
        def _():
            rows_start(wg_hbm, wg_v, msem.at[4], 0, D, WG_ROWS)
            rows_start(wu_hbm, wu_v, msem.at[5], 0, D, WG_ROWS)
            for c in range(NWD):
                rows_start(wd_hbm, wd_v, dsem.at[c], c * WD_GROUP, WD_GROUP, WD_ROWS)

        return slot

    x_copy = pltpu.make_async_copy(x_hbm, x_v, msem.at[0])
    wr_copy = pltpu.make_async_copy(wr_hbm, wr_v, msem.at[1])

    x_copy.start()
    wr_copy.start(priority=1)
    rows_start(wq_hbm, wq_v, msem.at[2], 0, D, WQ_ROWS)
    for u in range(LA):
        unit_start(u)

    x_copy.wait()
    x8_scr[...] = jnp.zeros((R, D), F32)
    x8_scr[0:B, :] = x_v[...].astype(F32)
    xn = _layernorm(x8_scr[...]).astype(BF)
    acc_scr[...] = jnp.zeros((R, D), F32)

    def head_mask(col0, width):
        row = lax.broadcasted_iota(jnp.int32, (H, width), 0)
        col = lax.broadcasted_iota(jnp.int32, (H, width), 1) + col0
        lo = row * DH
        return jnp.logical_and(col >= lo, col < lo + DH)

    wait_all(wq_v, msem.at[2])
    q_all = jnp.dot(xn, wq_v[...], preferred_element_type=F32)
    for rg in range(NRG):
        mask = head_mask(rg * GW, GW)
        for b in range(B):
            qrow = jnp.broadcast_to(q_all[b:b + 1, rg * GW:(rg + 1) * GW], (H, GW))
            qblk_scr[b * NRG + rg] = jnp.where(mask, qrow, 0.0).astype(BF)

    def batch(b, carry):
        u0 = b * (2 * UPB)
        s_scr[...] = jnp.zeros((H, SK), F32)

        def k_unit(t, c2):
            slot = advance(u0 + t)
            kt = buf[slot].reshape(GW, UC)
            col = pl.ds(pl.multiple_of((t % NCH) * UC, UC), UC)
            s_scr[:, col] += jnp.dot(qblk_scr[b * NRG + t // NCH], kt, preferred_element_type=F32)
            return c2

        lax.fori_loop(0, UPB, k_unit, 0)

        s = s_scr[...]
        m = jnp.max(s, axis=-1, keepdims=True)
        p = jnp.exp((s - m) * SCALE)
        l_scr[...] = jnp.sum(p, axis=-1, keepdims=True)
        p_scr[...] = p.astype(BF)

        def v_group(rg, c2):
            o_scr[...] = jnp.zeros((H, GW), F32)

            def v_unit(ch, c3):
                slot = advance(u0 + UPB + rg * NCH + ch)
                vt = buf[slot].reshape(GW, UC)
                col = pl.ds(pl.multiple_of(ch * UC, UC), UC)
                o_scr[...] += lax.dot_general(p_scr[:, col], vt, (((1,), (1,)), ((), ())),
                                              preferred_element_type=F32)
                return c3

            lax.fori_loop(0, NCH, v_unit, 0)

            @pl.when(jnp.logical_and(b == 0, rg == 0))
            def _():
                wait_all(wo_v, msem.at[3])

            ob = jnp.where(head_mask(rg * GW, GW), o_scr[...] / l_scr[...], 0.0).astype(BF)
            wo_g = wo_v[pl.ds(pl.multiple_of(rg * GW, GW), GW), :]
            contrib = jnp.sum(jnp.dot(ob, wo_g, preferred_element_type=F32), axis=0, keepdims=True)
            rows = lax.broadcasted_iota(jnp.int32, (R, D), 0)
            acc_scr[...] += jnp.where(rows == b, contrib, 0.0)
            return c2

        lax.fori_loop(0, NRG, v_group, 0)
        return carry

    lax.fori_loop(0, B, batch, 0)

    hres = x8_scr[...] + acc_scr[...]
    hn = _layernorm(hres)
    hb = hn.astype(BF)
    wr_copy.wait()
    wr = wr_v[...].astype(F32)
    racc = hn[:, 0:128] * wr[0:1, :]
    for j in range(1, D // 128):
        racc = racc + hn[:, j * 128:(j + 1) * 128] * wr[j:j + 1, :]
    gate = jax.nn.sigmoid(jnp.sum(racc, axis=-1, keepdims=True))
    base = hres + hn + hn * 0.0

    wait_all(wg_v, msem.at[4])
    g = jnp.dot(hb, wg_v[...], preferred_element_type=F32)
    g = g * jax.nn.sigmoid(g)
    wait_all(wu_v, msem.at[5])
    u = jnp.dot(hb, wu_v[...], preferred_element_type=F32)
    act = (g * u).astype(BF)
    y = None
    for c in range(NWD):
        rows_c = pl.ds(c * WD_GROUP, WD_GROUP)
        wait_all(wd_v.at[rows_c], dsem.at[c])
        part = jnp.dot(act[:, c * WD_GROUP:(c + 1) * WD_GROUP], wd_v[rows_c, :],
                       preferred_element_type=F32)
        y = part if y is None else y + part
    res = base + y * gate
    out_ref[...] = res[0:B, :].astype(BF)


@jax.jit
def pallas_sequential_preLN__mha_block_cached__moe_arch_mod__decode_kernel(
    A_x, A_k_cache, A_v_cache, A_wq, A_wo, B_x, B_w_r, B_w_gate, B_w_up, B_w_down,
):
    x2 = A_x.reshape(B, D)
    kt = jnp.swapaxes(A_k_cache, 2, 3).reshape(B * NRG, NA, NJ, 8, SK)
    vt = jnp.swapaxes(A_v_cache, 2, 3).reshape(B * NRG, NA, NJ, 8, SK)
    wr2 = B_w_r.reshape(D // 128, 128)
    any_spec = pl.BlockSpec(memory_space=pl.ANY)
    out = pl.pallas_call(
        _kernel,
        out_shape=jax.ShapeDtypeStruct((B, D), BF),
        in_specs=[any_spec] * 9,
        out_specs=pl.BlockSpec(memory_space=pltpu.VMEM),
        scratch_shapes=[
            pltpu.VMEM((B, D), BF),
            pltpu.VMEM((D // 128, 128), BF),
            pltpu.VMEM((D, H * DH), BF),
            pltpu.VMEM((H * DH, D), BF),
            pltpu.VMEM((D, F), BF),
            pltpu.VMEM((D, F), BF),
            pltpu.VMEM((F, D), BF),
            pltpu.VMEM((NSLOT, NA, NJ, 8, UC), BF),
            pltpu.VMEM((R, D), F32),
            pltpu.VMEM((B * NRG, H, GW), BF),
            pltpu.VMEM((H, SK), F32),
            pltpu.VMEM((H, SK), BF),
            pltpu.VMEM((H, 1), F32),
            pltpu.VMEM((H, GW), F32),
            pltpu.VMEM((R, D), F32),
            pltpu.SemaphoreType.DMA((NSLOT,)),
            pltpu.SemaphoreType.DMA((6,)),
            pltpu.SemaphoreType.DMA((NWD,)),
        ],
        compiler_params=pltpu.CompilerParams(vmem_limit_bytes=100 * 1024 * 1024),
    )(x2, kt, vt, A_wq, A_wo, wr2, B_w_gate, B_w_up, B_w_down)
    return out.reshape(B, 1, D)
```

```python
import jax
import jax.numpy as jnp
from jax import lax
import jax.experimental.pallas as pl
import jax.experimental.pallas.tpu as pltpu

B, D, H, SK, DH, F = 4, 640, 32, 8192, 192, 1536
HD = H * DH
R = 8

NA = 16
NJ = 16
GW = NA * NJ * 8
UC = 1024
CW = 128
NRG = HD // GW
NCH = SK // UC
UPB = NRG * NCH
NU = B * 2 * UPB
LA = 2
NSLOT = LA + 1

WQ_A, WQ_CW = 8, 256
WO_A, WO_CW = 12, 128
WG_ROWS = 32
WD_ROWS = 64
WD_GROUPS = (512, 512, 384, 128)
WD_OFF = tuple(sum(WD_GROUPS[:c]) for c in range(len(WD_GROUPS)))

EPS = 1e-5
SCALE = DH ** -0.5
BF = jnp.bfloat16
F32 = jnp.float32


def _layernorm(x):
    m = jnp.mean(x, axis=-1, keepdims=True)
    xc = x - m
    v = jnp.mean(xc * xc, axis=-1, keepdims=True)
    return xc / jnp.sqrt(v + EPS)


def _head_mask(col0, width):
    row = lax.broadcasted_iota(jnp.int32, (H, width), 0)
    col = lax.broadcasted_iota(jnp.int32, (H, width), 1) + col0
    lo = row * DH
    return jnp.logical_and(col >= lo, col < lo + DH)


def _kernel(x_hbm, k_hbm, v_hbm, wq_hbm, wo_hbm, wr_hbm, wg_hbm, wu_hbm, wd_hbm,
            out_ref,
            x_v, wr_v, wq_v, wo_v, wg_v, wu_v, wd_v, buf,
            x8_scr, qblk_scr, s_scr, p_scr, l_scr, o_scr, acc_scr,
            usem, msem, dsem):
    def unit_start_from(src, g, ch, slot):
        def issue(j, carry):
            for c in range(UC // CW):
                scol = pl.ds(pl.multiple_of(ch * UC + c * CW, CW), CW)
                pltpu.make_async_copy(src.at[g, :, j, :, scol],
                                      buf.at[slot, :, j, :, pl.ds(c * CW, CW)],
                                      usem.at[slot]).start(priority=c % 2)
            return carry

        lax.fori_loop(0, NJ, issue, 0)

    def unit_start(u):
        b = u // (2 * UPB)
        r = u % (2 * UPB)
        ru = r % UPB
        g = b * NRG + ru // NCH
        ch = ru % NCH
        slot = u % NSLOT

        @pl.when(r < UPB)
        def _():
            unit_start_from(k_hbm, g, ch, slot)

        @pl.when(r >= UPB)
        def _():
            unit_start_from(v_hbm, g, ch, slot)

    def strided_start(src, dst, sem, cw):
        nj, nc = src.shape[1], src.shape[3] // cw
        per = 1 if nc % 2 == 0 else 2

        def issue(jj, carry):
            for e in range(per):
                for c in range(nc):
                    j = jj * per + e
                    cols = pl.ds(c * cw, cw)
                    pltpu.make_async_copy(src.at[:, j, :, cols], dst.at[:, j, :, cols],
                                          sem).start(priority=(e * nc + c) % 2)
            return carry

        lax.fori_loop(0, nj // per, issue, 0)

    def rows_start(src, dst, sem, row0, nrows, step):
        def issue(c, carry):
            for j in range(2):
                rows = pl.ds(pl.multiple_of(row0 + (2 * c + j) * step, step), step)
                pltpu.make_async_copy(src.at[rows], dst.at[rows], sem).start(priority=j)
            return carry

        lax.fori_loop(0, nrows // (2 * step), issue, 0)

    def wait_all(dst, sem):
        pltpu.make_async_copy(dst, dst, sem).wait()

    def advance(u):
        slot = u % NSLOT
        wait_all(buf.at[slot], usem.at[slot])

        @pl.when(u == 0)
        def _():
            strided_start(wo_hbm, wo_v, msem.at[3], WO_CW)

        @pl.when(u + LA < NU)
        def _():
            unit_start(u + LA)

        @pl.when(u + LA == NU)
        def _():
            rows_start(wg_hbm, wg_v, msem.at[4], 0, D, WG_ROWS)
            rows_start(wu_hbm, wu_v, msem.at[5], 0, D, WG_ROWS)
            for c in range(len(WD_GROUPS)):
                rows_start(wd_hbm, wd_v, dsem.at[c], WD_OFF[c], WD_GROUPS[c], WD_ROWS)

        return slot

    x_copy = pltpu.make_async_copy(x_hbm, x_v, msem.at[0])
    wr_copy = pltpu.make_async_copy(wr_hbm, wr_v, msem.at[1])

    strided_start(wq_hbm, wq_v, msem.at[2], WQ_CW)
    x_copy.start()
    wr_copy.start(priority=1)
    for u in range(LA):
        unit_start(u)

    x_copy.wait()
    x8_scr[...] = jnp.zeros((R, D), F32)
    x8_scr[0:B, :] = x_v[...].astype(F32)
    xn = _layernorm(x8_scr[...]).astype(BF)
    acc_scr[...] = jnp.zeros((R, D), F32)

    wait_all(wq_v, msem.at[2])
    q_all = jnp.dot(xn, wq_v[...].reshape(D, HD), preferred_element_type=F32)
    for rg in range(NRG):
        mask = _head_mask(rg * GW, GW)
        for b in range(B):
            qrow = jnp.broadcast_to(q_all[b:b + 1, rg * GW:(rg + 1) * GW], (H, GW))
            qblk_scr[b * NRG + rg] = jnp.where(mask, qrow, 0.0).astype(BF)

    def batch(b, carry):
        u0 = b * (2 * UPB)
        s_scr[...] = jnp.zeros((H, SK), F32)

        def k_unit(t, c2):
            slot = advance(u0 + t)
            kt = buf[slot].reshape(GW, UC)
            col = pl.ds(pl.multiple_of((t % NCH) * UC, UC), UC)
            s_scr[:, col] += jnp.dot(qblk_scr[b * NRG + t // NCH], kt, preferred_element_type=F32)
            return c2

        lax.fori_loop(0, UPB, k_unit, 0)

        s = s_scr[...]
        m = jnp.max(s, axis=-1, keepdims=True)
        p = jnp.exp((s - m) * SCALE)
        l_scr[...] = jnp.sum(p, axis=-1, keepdims=True)
        p_scr[...] = p.astype(BF)

        def v_group(rg, c2):
            o_scr[...] = jnp.zeros((H, GW), F32)

            def v_unit(ch, c3):
                slot = advance(u0 + UPB + rg * NCH + ch)
                vt = buf[slot].reshape(GW, UC)
                col = pl.ds(pl.multiple_of(ch * UC, UC), UC)
                o_scr[...] += lax.dot_general(p_scr[:, col], vt, (((1,), (1,)), ((), ())),
                                              preferred_element_type=F32)
                return c3

            lax.fori_loop(0, NCH, v_unit, 0)

            @pl.when(jnp.logical_and(b == 0, rg == 0))
            def _():
                wait_all(wo_v, msem.at[3])

            ob = jnp.where(_head_mask(rg * GW, GW), o_scr[...] / l_scr[...], 0.0).astype(BF)
            wo_g = wo_v[pl.ds(rg * (WO_A // NRG), WO_A // NRG)].reshape(GW, D)
            contrib = jnp.sum(jnp.dot(ob, wo_g, preferred_element_type=F32), axis=0, keepdims=True)
            rows = lax.broadcasted_iota(jnp.int32, (R, D), 0)
            acc_scr[...] += jnp.where(rows == b, contrib, 0.0)
            return c2

        lax.fori_loop(0, NRG, v_group, 0)
        return carry

    lax.fori_loop(0, B, batch, 0)

    hres = x8_scr[...] + acc_scr[...]
    hn = _layernorm(hres)
    hb = hn.astype(BF)
    wr_copy.wait()
    wr = wr_v[...].astype(F32)
    racc = hn[:, 0:128] * wr[0:1, :]
    for j in range(1, D // 128):
        racc = racc + hn[:, j * 128:(j + 1) * 128] * wr[j:j + 1, :]
    gate = jax.nn.sigmoid(jnp.sum(racc, axis=-1, keepdims=True))
    base = hres + hn + hn * 0.0

    wait_all(wg_v, msem.at[4])
    g = jnp.dot(hb, wg_v[...], preferred_element_type=F32)
    g = g * jax.nn.sigmoid(g)
    wait_all(wu_v, msem.at[5])
    u = jnp.dot(hb, wu_v[...], preferred_element_type=F32)
    act = (g * u).astype(BF)
    y = None
    for c in range(len(WD_GROUPS)):
        rows_c = pl.ds(WD_OFF[c], WD_GROUPS[c])
        wait_all(wd_v.at[rows_c], dsem.at[c])
        part = jnp.dot(act[:, WD_OFF[c]:WD_OFF[c] + WD_GROUPS[c]], wd_v[rows_c, :],
                       preferred_element_type=F32)
        y = part if y is None else y + part
    res = base + y * gate
    out_ref[...] = res[0:B, :].astype(BF)


@jax.jit
def pallas_sequential_preLN__mha_block_cached__moe_arch_mod__decode_kernel(
    A_x, A_k_cache, A_v_cache, A_wq, A_wo, B_x, B_w_r, B_w_gate, B_w_up, B_w_down,
):
    x2 = A_x.reshape(B, D)
    kt = jnp.swapaxes(A_k_cache, 2, 3).reshape(B * NRG, NA, NJ, 8, SK)
    vt = jnp.swapaxes(A_v_cache, 2, 3).reshape(B * NRG, NA, NJ, 8, SK)
    wq4 = A_wq.reshape(WQ_A, D // 8 // WQ_A, 8, HD)
    wo4 = A_wo.reshape(WO_A, HD // 8 // WO_A, 8, D)
    wr2 = B_w_r.reshape(D // 128, 128)
    any_spec = pl.BlockSpec(memory_space=pl.ANY)
    out = pl.pallas_call(
        _kernel,
        out_shape=jax.ShapeDtypeStruct((B, D), BF),
        in_specs=[any_spec] * 9,
        out_specs=pl.BlockSpec(memory_space=pltpu.VMEM),
        scratch_shapes=[
            pltpu.VMEM((B, D), BF),
            pltpu.VMEM((D // 128, 128), BF),
            pltpu.VMEM((WQ_A, D // 8 // WQ_A, 8, HD), BF),
            pltpu.VMEM((WO_A, HD // 8 // WO_A, 8, D), BF),
            pltpu.VMEM((D, F), BF),
            pltpu.VMEM((D, F), BF),
            pltpu.VMEM((F, D), BF),
            pltpu.VMEM((NSLOT, NA, NJ, 8, UC), BF),
            pltpu.VMEM((R, D), F32),
            pltpu.VMEM((B * NRG, H, GW), BF),
            pltpu.VMEM((H, SK), F32),
            pltpu.VMEM((H, SK), BF),
            pltpu.VMEM((H, 1), F32),
            pltpu.VMEM((H, GW), F32),
            pltpu.VMEM((R, D), F32),
            pltpu.SemaphoreType.DMA((NSLOT,)),
            pltpu.SemaphoreType.DMA((6,)),
            pltpu.SemaphoreType.DMA((len(WD_GROUPS),)),
        ],
        compiler_params=pltpu.CompilerParams(vmem_limit_bytes=100 * 1024 * 1024),
    )(x2, kt, vt, wq4, wo4, wr2, B_w_gate, B_w_up, B_w_down)
    return out.reshape(B, 1, D)
```

```python
import jax
import jax.numpy as jnp
from jax import lax
import jax.experimental.pallas as pl
import jax.experimental.pallas.tpu as pltpu

B, D, H, SK, DH, F = 4, 640, 32, 8192, 192, 1536
HD = H * DH
R = 8

NA = 8
NJ = 16
GW = NA * NJ * 8
UC = 2048
CW = 256
NRG = HD // GW
NCH = SK // UC
UPB = NRG * NCH
NU = B * 2 * UPB
LA = 2
NSLOT = LA + 1

WQ_A, WQ_CW = 8, 256
WO_A, WO_CW = 12, 128
WG_ROWS = 32
WD_ROWS = 64
WD_GROUPS = (512, 512, 384, 128)
WD_OFF = tuple(sum(WD_GROUPS[:c]) for c in range(len(WD_GROUPS)))

EPS = 1e-5
SCALE = DH ** -0.5
BF = jnp.bfloat16
F32 = jnp.float32


def _layernorm(x):
    m = jnp.mean(x, axis=-1, keepdims=True)
    xc = x - m
    v = jnp.mean(xc * xc, axis=-1, keepdims=True)
    return xc / jnp.sqrt(v + EPS)


def _head_mask(col0, width):
    row = lax.broadcasted_iota(jnp.int32, (H, width), 0)
    col = lax.broadcasted_iota(jnp.int32, (H, width), 1) + col0
    lo = row * DH
    return jnp.logical_and(col >= lo, col < lo + DH)


def _kernel(x_hbm, k_hbm, v_hbm, wq_hbm, wo_hbm, wr_hbm, wg_hbm, wu_hbm, wd_hbm,
            out_ref,
            x_v, wr_v, wq_v, wo_v, wg_v, wu_v, wd_v, buf,
            x8_scr, qblk_scr, s_scr, p_scr, l_scr, o_scr, acc_scr,
            usem, msem, dsem):
    def unit_start_from(src, g, ch, slot):
        nc = UC // CW

        def issue(j, carry):
            for c in range(nc // 2):
                for e in range(2):
                    cc = c + e * (nc // 2)
                    scol = pl.ds(pl.multiple_of(ch * UC + cc * CW, CW), CW)
                    pltpu.make_async_copy(src.at[g, :, j, :, scol],
                                          buf.at[slot, :, j, :, pl.ds(cc * CW, CW)],
                                          usem.at[slot]).start(priority=e)
            return carry

        lax.fori_loop(0, NJ, issue, 0)

    def unit_start(u):
        b = u // (2 * UPB)
        r = u % (2 * UPB)
        ru = r % UPB
        g = b * NRG + ru // NCH
        ch = ru % NCH
        slot = u % NSLOT

        @pl.when(r < UPB)
        def _():
            unit_start_from(k_hbm, g, ch, slot)

        @pl.when(r >= UPB)
        def _():
            unit_start_from(v_hbm, g, ch, slot)

    def strided_start(src, dst, sem, cw):
        nj, nc = src.shape[1], src.shape[3] // cw
        per = 1 if nc % 2 == 0 else 2

        def issue(jj, carry):
            for e in range(per):
                for c in range(nc):
                    j = jj * per + e
                    cols = pl.ds(c * cw, cw)
                    pltpu.make_async_copy(src.at[:, j, :, cols], dst.at[:, j, :, cols],
                                          sem).start(priority=(e * nc + c) % 2)
            return carry

        lax.fori_loop(0, nj // per, issue, 0)

    def rows_start(src, dst, sem, row0, nrows, step):
        def issue(c, carry):
            for j in range(2):
                rows = pl.ds(pl.multiple_of(row0 + (2 * c + j) * step, step), step)
                pltpu.make_async_copy(src.at[rows], dst.at[rows], sem).start(priority=j)
            return carry

        lax.fori_loop(0, nrows // (2 * step), issue, 0)

    def wait_all(dst, sem):
        pltpu.make_async_copy(dst, dst, sem).wait()

    def advance(u):
        slot = u % NSLOT
        wait_all(buf.at[slot], usem.at[slot])

        @pl.when(u == 0)
        def _():
            strided_start(wo_hbm, wo_v, msem.at[3], WO_CW)

        @pl.when(u + LA < NU)
        def _():
            unit_start(u + LA)

        @pl.when(u + LA == NU)
        def _():
            rows_start(wg_hbm, wg_v, msem.at[4], 0, D, WG_ROWS)
            rows_start(wu_hbm, wu_v, msem.at[5], 0, D, WG_ROWS)
            for c in range(len(WD_GROUPS)):
                rows_start(wd_hbm, wd_v, dsem.at[c], WD_OFF[c], WD_GROUPS[c], WD_ROWS)

        return slot

    x_copy = pltpu.make_async_copy(x_hbm, x_v, msem.at[0])
    wr_copy = pltpu.make_async_copy(wr_hbm, wr_v, msem.at[1])

    strided_start(wq_hbm, wq_v, msem.at[2], WQ_CW)
    x_copy.start()
    wr_copy.start(priority=1)
    for u in range(LA):
        unit_start(u)

    x_copy.wait()
    x8_scr[...] = jnp.zeros((R, D), F32)
    x8_scr[0:B, :] = x_v[...].astype(F32)
    xn = _layernorm(x8_scr[...]).astype(BF)
    acc_scr[...] = jnp.zeros((R, D), F32)

    wait_all(wq_v, msem.at[2])
    q_all = jnp.dot(xn, wq_v[...].reshape(D, HD), preferred_element_type=F32)
    for rg in range(NRG):
        mask = _head_mask(rg * GW, GW)
        for b in range(B):
            qrow = jnp.broadcast_to(q_all[b:b + 1, rg * GW:(rg + 1) * GW], (H, GW))
            qblk_scr[b * NRG + rg] = jnp.where(mask, qrow, 0.0).astype(BF)

    def batch(b, carry):
        u0 = b * (2 * UPB)
        s_scr[...] = jnp.zeros((H, SK), F32)

        def k_unit(t, c2):
            slot = advance(u0 + t)
            kt = buf[slot].reshape(GW, UC)
            col = pl.ds(pl.multiple_of((t % NCH) * UC, UC), UC)
            s_scr[:, col] += jnp.dot(qblk_scr[b * NRG + t // NCH], kt, preferred_element_type=F32)
            return c2

        lax.fori_loop(0, UPB, k_unit, 0)

        s = s_scr[...]
        m = jnp.max(s, axis=-1, keepdims=True)
        p = jnp.exp((s - m) * SCALE)
        l_scr[...] = jnp.sum(p, axis=-1, keepdims=True)
        p_scr[...] = p.astype(BF)

        def v_group(rg, c2):
            o_scr[...] = jnp.zeros((H, GW), F32)

            def v_unit(ch, c3):
                slot = advance(u0 + UPB + rg * NCH + ch)
                vt = buf[slot].reshape(GW, UC)
                col = pl.ds(pl.multiple_of(ch * UC, UC), UC)
                o_scr[...] += lax.dot_general(p_scr[:, col], vt, (((1,), (1,)), ((), ())),
                                              preferred_element_type=F32)
                return c3

            lax.fori_loop(0, NCH, v_unit, 0)

            @pl.when(jnp.logical_and(b == 0, rg == 0))
            def _():
                wait_all(wo_v, msem.at[3])

            ob = jnp.where(_head_mask(rg * GW, GW), o_scr[...] / l_scr[...], 0.0).astype(BF)
            wo_g = wo_v[pl.ds(rg * (WO_A // NRG), WO_A // NRG)].reshape(GW, D)
            contrib = jnp.sum(jnp.dot(ob, wo_g, preferred_element_type=F32), axis=0, keepdims=True)
            rows = lax.broadcasted_iota(jnp.int32, (R, D), 0)
            acc_scr[...] += jnp.where(rows == b, contrib, 0.0)
            return c2

        lax.fori_loop(0, NRG, v_group, 0)
        return carry

    lax.fori_loop(0, B, batch, 0)

    hres = x8_scr[...] + acc_scr[...]
    hn = _layernorm(hres)
    hb = hn.astype(BF)
    wr_copy.wait()
    wr = wr_v[...].astype(F32)
    racc = hn[:, 0:128] * wr[0:1, :]
    for j in range(1, D // 128):
        racc = racc + hn[:, j * 128:(j + 1) * 128] * wr[j:j + 1, :]
    gate = jax.nn.sigmoid(jnp.sum(racc, axis=-1, keepdims=True))
    base = hres + hn + hn * 0.0

    wait_all(wg_v, msem.at[4])
    g = jnp.dot(hb, wg_v[...], preferred_element_type=F32)
    g = g * jax.nn.sigmoid(g)
    wait_all(wu_v, msem.at[5])
    u = jnp.dot(hb, wu_v[...], preferred_element_type=F32)
    act = (g * u).astype(BF)
    y = None
    for c in range(len(WD_GROUPS)):
        rows_c = pl.ds(WD_OFF[c], WD_GROUPS[c])
        wait_all(wd_v.at[rows_c], dsem.at[c])
        part = jnp.dot(act[:, WD_OFF[c]:WD_OFF[c] + WD_GROUPS[c]], wd_v[rows_c, :],
                       preferred_element_type=F32)
        y = part if y is None else y + part
    res = base + y * gate
    out_ref[...] = res[0:B, :].astype(BF)


@jax.jit
def pallas_sequential_preLN__mha_block_cached__moe_arch_mod__decode_kernel(
    A_x, A_k_cache, A_v_cache, A_wq, A_wo, B_x, B_w_r, B_w_gate, B_w_up, B_w_down,
):
    x2 = A_x.reshape(B, D)
    kt = jnp.swapaxes(A_k_cache, 2, 3).reshape(B * NRG, NA, NJ, 8, SK)
    vt = jnp.swapaxes(A_v_cache, 2, 3).reshape(B * NRG, NA, NJ, 8, SK)
    wq4 = A_wq.reshape(WQ_A, D // 8 // WQ_A, 8, HD)
    wo4 = A_wo.reshape(WO_A, HD // 8 // WO_A, 8, D)
    wr2 = B_w_r.reshape(D // 128, 128)
    any_spec = pl.BlockSpec(memory_space=pl.ANY)
    out = pl.pallas_call(
        _kernel,
        out_shape=jax.ShapeDtypeStruct((B, D), BF),
        in_specs=[any_spec] * 9,
        out_specs=pl.BlockSpec(memory_space=pltpu.VMEM),
        scratch_shapes=[
            pltpu.VMEM((B, D), BF),
            pltpu.VMEM((D // 128, 128), BF),
            pltpu.VMEM((WQ_A, D // 8 // WQ_A, 8, HD), BF),
            pltpu.VMEM((WO_A, HD // 8 // WO_A, 8, D), BF),
            pltpu.VMEM((D, F), BF),
            pltpu.VMEM((D, F), BF),
            pltpu.VMEM((F, D), BF),
            pltpu.VMEM((NSLOT, NA, NJ, 8, UC), BF),
            pltpu.VMEM((R, D), F32),
            pltpu.VMEM((B * NRG, H, GW), BF),
            pltpu.VMEM((H, SK), F32),
            pltpu.VMEM((H, SK), BF),
            pltpu.VMEM((H, 1), F32),
            pltpu.VMEM((H, GW), F32),
            pltpu.VMEM((R, D), F32),
            pltpu.SemaphoreType.DMA((NSLOT,)),
            pltpu.SemaphoreType.DMA((6,)),
            pltpu.SemaphoreType.DMA((len(WD_GROUPS),)),
        ],
        compiler_params=pltpu.CompilerParams(vmem_limit_bytes=100 * 1024 * 1024),
    )(x2, kt, vt, wq4, wo4, wr2, B_w_gate, B_w_up, B_w_down)
    return out.reshape(B, 1, D)
```

```python
import jax
import jax.numpy as jnp
from jax import lax
import jax.experimental.pallas as pl
import jax.experimental.pallas.tpu as pltpu

B, D, H, SK, DH, F = 4, 640, 32, 8192, 192, 1536
HD = H * DH
R = 8

NA = 2
NJ = 64
SJ = 8
GW = NA * NJ * 8
UC = 2048
CW = 1024
NRG = HD // GW
NCH = SK // UC
UPB = NRG * NCH
NU = B * 2 * UPB
LA = 2
NSLOT = LA + 1

WQ_A, WQ_CW = 8, 256
WO_A, WO_CW = 12, 128
WG_ROWS = 32
WD_ROWS = 64
WD_GROUPS = (512, 512, 384, 128)
WD_OFF = tuple(sum(WD_GROUPS[:c]) for c in range(len(WD_GROUPS)))

EPS = 1e-5
SCALE = DH ** -0.5
BF = jnp.bfloat16
F32 = jnp.float32


def _layernorm(x):
    m = jnp.mean(x, axis=-1, keepdims=True)
    xc = x - m
    v = jnp.mean(xc * xc, axis=-1, keepdims=True)
    return xc / jnp.sqrt(v + EPS)


def _head_mask(col0, width):
    row = lax.broadcasted_iota(jnp.int32, (H, width), 0)
    col = lax.broadcasted_iota(jnp.int32, (H, width), 1) + col0
    lo = row * DH
    return jnp.logical_and(col >= lo, col < lo + DH)


def _kernel(x_hbm, k_hbm, v_hbm, wq_hbm, wo_hbm, wr_hbm, wg_hbm, wu_hbm, wd_hbm,
            out_ref,
            x_v, wr_v, wq_v, wo_v, wg_v, wu_v, wd_v, buf,
            x8_scr, qblk_scr, s_scr, p_scr, l_scr, o_scr, acc_scr,
            usem, msem, dsem):
    def unit_start_from(src, g, ch, slot):
        def issue(jj, carry):
            for c in range(UC // CW):
                scol = pl.ds(pl.multiple_of(ch * UC + c * CW, CW), CW)
                for a in range(NJ // SJ):
                    j = a * SJ + jj
                    pltpu.make_async_copy(src.at[g, :, j, :, scol],
                                          buf.at[slot, :, j, :, pl.ds(c * CW, CW)],
                                          usem.at[slot]).start(priority=a % 2)
            return carry

        lax.fori_loop(0, SJ, issue, 0)

    def unit_start(u):
        b = u // (2 * UPB)
        r = u % (2 * UPB)
        ru = r % UPB
        g = b * NRG + ru // NCH
        ch = ru % NCH
        slot = u % NSLOT

        @pl.when(r < UPB)
        def _():
            unit_start_from(k_hbm, g, ch, slot)

        @pl.when(r >= UPB)
        def _():
            unit_start_from(v_hbm, g, ch, slot)

    def strided_start(src, dst, sem, cw):
        nj, nc = src.shape[1], src.shape[3] // cw
        per = 1 if nc % 2 == 0 else 2

        def issue(jj, carry):
            for e in range(per):
                for c in range(nc):
                    j = jj * per + e
                    cols = pl.ds(c * cw, cw)
                    pltpu.make_async_copy(src.at[:, j, :, cols], dst.at[:, j, :, cols],
                                          sem).start(priority=(e * nc + c) % 2)
            return carry

        lax.fori_loop(0, nj // per, issue, 0)

    def rows_start(src, dst, sem, row0, nrows, step):
        def issue(c, carry):
            for j in range(2):
                rows = pl.ds(pl.multiple_of(row0 + (2 * c + j) * step, step), step)
                pltpu.make_async_copy(src.at[rows], dst.at[rows], sem).start(priority=j)
            return carry

        lax.fori_loop(0, nrows // (2 * step), issue, 0)

    def wait_all(dst, sem):
        pltpu.make_async_copy(dst, dst, sem).wait()

    def advance(u):
        slot = u % NSLOT
        wait_all(buf.at[slot], usem.at[slot])

        @pl.when(u == 0)
        def _():
            strided_start(wo_hbm, wo_v, msem.at[3], WO_CW)

        @pl.when(u + LA < NU)
        def _():
            unit_start(u + LA)

        @pl.when(u + LA == NU)
        def _():
            rows_start(wg_hbm, wg_v, msem.at[4], 0, D, WG_ROWS)
            rows_start(wu_hbm, wu_v, msem.at[5], 0, D, WG_ROWS)
            for c in range(len(WD_GROUPS)):
                rows_start(wd_hbm, wd_v, dsem.at[c], WD_OFF[c], WD_GROUPS[c], WD_ROWS)

        return slot

    x_copy = pltpu.make_async_copy(x_hbm, x_v, msem.at[0])
    wr_copy = pltpu.make_async_copy(wr_hbm, wr_v, msem.at[1])

    strided_start(wq_hbm, wq_v, msem.at[2], WQ_CW)
    x_copy.start()
    wr_copy.start(priority=1)
    for u in range(LA):
        unit_start(u)

    x_copy.wait()
    x8_scr[...] = jnp.zeros((R, D), F32)
    x8_scr[0:B, :] = x_v[...].astype(F32)
    xn = _layernorm(x8_scr[...]).astype(BF)
    acc_scr[...] = jnp.zeros((R, D), F32)

    wait_all(wq_v, msem.at[2])
    q_all = jnp.dot(xn, wq_v[...].reshape(D, HD), preferred_element_type=F32)
    for rg in range(NRG):
        mask = _head_mask(rg * GW, GW)
        for b in range(B):
            qrow = jnp.broadcast_to(q_all[b:b + 1, rg * GW:(rg + 1) * GW], (H, GW))
            qblk_scr[b * NRG + rg] = jnp.where(mask, qrow, 0.0).astype(BF)

    def batch(b, carry):
        u0 = b * (2 * UPB)
        s_scr[...] = jnp.zeros((H, SK), F32)

        def k_unit(t, c2):
            slot = advance(u0 + t)
            kt = buf[slot].reshape(GW, UC)
            col = pl.ds(pl.multiple_of((t % NCH) * UC, UC), UC)
            s_scr[:, col] += jnp.dot(qblk_scr[b * NRG + t // NCH], kt, preferred_element_type=F32)
            return c2

        lax.fori_loop(0, UPB, k_unit, 0)

        s = s_scr[...]
        m = jnp.max(s, axis=-1, keepdims=True)
        p = jnp.exp((s - m) * SCALE)
        l_scr[...] = jnp.sum(p, axis=-1, keepdims=True)
        p_scr[...] = p.astype(BF)

        def v_group(rg, c2):
            o_scr[...] = jnp.zeros((H, GW), F32)

            def v_unit(ch, c3):
                slot = advance(u0 + UPB + rg * NCH + ch)
                vt = buf[slot].reshape(GW, UC)
                col = pl.ds(pl.multiple_of(ch * UC, UC), UC)
                o_scr[...] += lax.dot_general(p_scr[:, col], vt, (((1,), (1,)), ((), ())),
                                              preferred_element_type=F32)
                return c3

            lax.fori_loop(0, NCH, v_unit, 0)

            @pl.when(jnp.logical_and(b == 0, rg == 0))
            def _():
                wait_all(wo_v, msem.at[3])

            ob = jnp.where(_head_mask(rg * GW, GW), o_scr[...] / l_scr[...], 0.0).astype(BF)
            wo_g = wo_v[pl.ds(rg * (WO_A // NRG), WO_A // NRG)].reshape(GW, D)
            contrib = jnp.sum(jnp.dot(ob, wo_g, preferred_element_type=F32), axis=0, keepdims=True)
            rows = lax.broadcasted_iota(jnp.int32, (R, D), 0)
            acc_scr[...] += jnp.where(rows == b, contrib, 0.0)
            return c2

        lax.fori_loop(0, NRG, v_group, 0)
        return carry

    lax.fori_loop(0, B, batch, 0)

    hres = x8_scr[...] + acc_scr[...]
    hn = _layernorm(hres)
    hb = hn.astype(BF)
    wr_copy.wait()
    wr = wr_v[...].astype(F32)
    racc = hn[:, 0:128] * wr[0:1, :]
    for j in range(1, D // 128):
        racc = racc + hn[:, j * 128:(j + 1) * 128] * wr[j:j + 1, :]
    gate = jax.nn.sigmoid(jnp.sum(racc, axis=-1, keepdims=True))
    base = hres + hn + hn * 0.0

    wait_all(wg_v, msem.at[4])
    g = jnp.dot(hb, wg_v[...], preferred_element_type=F32)
    g = g * jax.nn.sigmoid(g)
    wait_all(wu_v, msem.at[5])
    u = jnp.dot(hb, wu_v[...], preferred_element_type=F32)
    act = (g * u).astype(BF)
    y = None
    for c in range(len(WD_GROUPS)):
        rows_c = pl.ds(WD_OFF[c], WD_GROUPS[c])
        wait_all(wd_v.at[rows_c], dsem.at[c])
        part = jnp.dot(act[:, WD_OFF[c]:WD_OFF[c] + WD_GROUPS[c]], wd_v[rows_c, :],
                       preferred_element_type=F32)
        y = part if y is None else y + part
    res = base + y * gate
    out_ref[...] = res[0:B, :].astype(BF)


@jax.jit
def pallas_sequential_preLN__mha_block_cached__moe_arch_mod__decode_kernel(
    A_x, A_k_cache, A_v_cache, A_wq, A_wo, B_x, B_w_r, B_w_gate, B_w_up, B_w_down,
):
    x2 = A_x.reshape(B, D)
    kt = jnp.swapaxes(A_k_cache, 2, 3).reshape(B * NRG, NA, NJ, 8, SK)
    vt = jnp.swapaxes(A_v_cache, 2, 3).reshape(B * NRG, NA, NJ, 8, SK)
    wq4 = A_wq.reshape(WQ_A, D // 8 // WQ_A, 8, HD)
    wo4 = A_wo.reshape(WO_A, HD // 8 // WO_A, 8, D)
    wr2 = B_w_r.reshape(D // 128, 128)
    any_spec = pl.BlockSpec(memory_space=pl.ANY)
    out = pl.pallas_call(
        _kernel,
        out_shape=jax.ShapeDtypeStruct((B, D), BF),
        in_specs=[any_spec] * 9,
        out_specs=pl.BlockSpec(memory_space=pltpu.VMEM),
        scratch_shapes=[
            pltpu.VMEM((B, D), BF),
            pltpu.VMEM((D // 128, 128), BF),
            pltpu.VMEM((WQ_A, D // 8 // WQ_A, 8, HD), BF),
            pltpu.VMEM((WO_A, HD // 8 // WO_A, 8, D), BF),
            pltpu.VMEM((D, F), BF),
            pltpu.VMEM((D, F), BF),
            pltpu.VMEM((F, D), BF),
            pltpu.VMEM((NSLOT, NA, NJ, 8, UC), BF),
            pltpu.VMEM((R, D), F32),
            pltpu.VMEM((B * NRG, H, GW), BF),
            pltpu.VMEM((H, SK), F32),
            pltpu.VMEM((H, SK), BF),
            pltpu.VMEM((H, 1), F32),
            pltpu.VMEM((H, GW), F32),
            pltpu.VMEM((R, D), F32),
            pltpu.SemaphoreType.DMA((NSLOT,)),
            pltpu.SemaphoreType.DMA((6,)),
            pltpu.SemaphoreType.DMA((len(WD_GROUPS),)),
        ],
        compiler_params=pltpu.CompilerParams(vmem_limit_bytes=100 * 1024 * 1024),
    )(x2, kt, vt, wq4, wo4, wr2, B_w_gate, B_w_up, B_w_down)
    return out.reshape(B, 1, D)
```

```python
import jax
import jax.numpy as jnp
from jax import lax
import jax.experimental.pallas as pl
import jax.experimental.pallas.tpu as pltpu

B, D, H, SK, DH, F = 4, 640, 32, 8192, 192, 1536
HD = H * DH
R = 8

NA = 2
NJ = 64
SJ = 8
GW = NA * NJ * 8
UC = 2048
CW = 1024
NRG = HD // GW
NCH = SK // UC
UPB = NRG * NCH
NU = B * 2 * UPB
LA = 2
NSLOT = LA + 1

WQ_BLK = (8, 2048)
WO_BLK = (24, D)
WG_BLK = (16, F)
W_WAYS = 8
WD_ROWS = 64
WD_GROUPS = (512, 512, 384, 128)
WD_OFF = tuple(sum(WD_GROUPS[:c]) for c in range(len(WD_GROUPS)))

EPS = 1e-5
SCALE = DH ** -0.5
BF = jnp.bfloat16
F32 = jnp.float32


def _layernorm(x):
    m = jnp.mean(x, axis=-1, keepdims=True)
    xc = x - m
    v = jnp.mean(xc * xc, axis=-1, keepdims=True)
    return xc / jnp.sqrt(v + EPS)


def _head_mask(col0, width):
    row = lax.broadcasted_iota(jnp.int32, (H, width), 0)
    col = lax.broadcasted_iota(jnp.int32, (H, width), 1) + col0
    lo = row * DH
    return jnp.logical_and(col >= lo, col < lo + DH)


def _kernel(x_hbm, k_hbm, v_hbm, wq_hbm, wo_hbm, wr_hbm, wg_hbm, wu_hbm, wd_hbm,
            out_ref,
            x_v, wr_v, wq_v, wo_v, wg_v, wu_v, wd_v, buf,
            x8_scr, qblk_scr, s_scr, p_scr, l_scr, o_scr, acc_scr,
            usem, msem, dsem):
    def unit_start_from(src, g, ch, slot):
        def issue(jj, carry):
            for c in range(UC // CW):
                scol = pl.ds(pl.multiple_of(ch * UC + c * CW, CW), CW)
                for a in range(NJ // SJ):
                    j = a * SJ + jj
                    pltpu.make_async_copy(src.at[g, :, j, :, scol],
                                          buf.at[slot, :, j, :, pl.ds(c * CW, CW)],
                                          usem.at[slot]).start(priority=a % 2)
            return carry

        lax.fori_loop(0, SJ, issue, 0)

    def unit_start(u):
        b = u // (2 * UPB)
        r = u % (2 * UPB)
        ru = r % UPB
        g = b * NRG + ru // NCH
        ch = ru % NCH
        slot = u % NSLOT

        @pl.when(r < UPB)
        def _():
            unit_start_from(k_hbm, g, ch, slot)

        @pl.when(r >= UPB)
        def _():
            unit_start_from(v_hbm, g, ch, slot)

    def blocks_start(src, dst, sem, blk):
        rr, cc = blk
        s1 = src.shape[0] // rr // W_WAYS

        def issue(jj, carry):
            for c in range(src.shape[1] // cc):
                for a in range(W_WAYS):
                    rows = pl.ds(pl.multiple_of((a * s1 + jj) * rr, 8), rr)
                    cols = pl.ds(c * cc, cc)
                    pltpu.make_async_copy(src.at[rows, cols], dst.at[rows, cols],
                                          sem).start(priority=a % 2)
            return carry

        lax.fori_loop(0, s1, issue, 0)

    def rows_start(src, dst, sem, row0, nrows, step):
        def issue(c, carry):
            for j in range(2):
                rows = pl.ds(pl.multiple_of(row0 + (2 * c + j) * step, step), step)
                pltpu.make_async_copy(src.at[rows], dst.at[rows], sem).start(priority=j)
            return carry

        lax.fori_loop(0, nrows // (2 * step), issue, 0)

    def wait_all(dst, sem):
        pltpu.make_async_copy(dst, dst, sem).wait()

    def advance(u):
        slot = u % NSLOT
        wait_all(buf.at[slot], usem.at[slot])

        @pl.when(u == 0)
        def _():
            blocks_start(wo_hbm, wo_v, msem.at[3], WO_BLK)

        @pl.when(u + LA < NU)
        def _():
            unit_start(u + LA)

        @pl.when(u + LA == NU)
        def _():
            blocks_start(wg_hbm, wg_v, msem.at[4], WG_BLK)
            blocks_start(wu_hbm, wu_v, msem.at[5], WG_BLK)
            for c in range(len(WD_GROUPS)):
                rows_start(wd_hbm, wd_v, dsem.at[c], WD_OFF[c], WD_GROUPS[c], WD_ROWS)

        return slot

    x_copy = pltpu.make_async_copy(x_hbm, x_v, msem.at[0])
    wr_copy = pltpu.make_async_copy(wr_hbm, wr_v, msem.at[1])

    blocks_start(wq_hbm, wq_v, msem.at[2], WQ_BLK)
    x_copy.start()
    wr_copy.start(priority=1)
    for u in range(LA):
        unit_start(u)

    x_copy.wait()
    x8_scr[...] = jnp.zeros((R, D), F32)
    x8_scr[0:B, :] = x_v[...].astype(F32)
    xn = _layernorm(x8_scr[...]).astype(BF)
    acc_scr[...] = jnp.zeros((R, D), F32)

    wait_all(wq_v, msem.at[2])
    q_all = jnp.dot(xn, wq_v[...], preferred_element_type=F32)
    for rg in range(NRG):
        mask = _head_mask(rg * GW, GW)
        for b in range(B):
            qrow = jnp.broadcast_to(q_all[b:b + 1, rg * GW:(rg + 1) * GW], (H, GW))
            qblk_scr[b * NRG + rg] = jnp.where(mask, qrow, 0.0).astype(BF)

    def batch(b, carry):
        u0 = b * (2 * UPB)
        s_scr[...] = jnp.zeros((H, SK), F32)

        def k_unit(t, c2):
            slot = advance(u0 + t)
            kt = buf[slot].reshape(GW, UC)
            col = pl.ds(pl.multiple_of((t % NCH) * UC, UC), UC)
            s_scr[:, col] += jnp.dot(qblk_scr[b * NRG + t // NCH], kt, preferred_element_type=F32)
            return c2

        lax.fori_loop(0, UPB, k_unit, 0)

        s = s_scr[...]
        m = jnp.max(s, axis=-1, keepdims=True)
        p = jnp.exp((s - m) * SCALE)
        l_scr[...] = jnp.sum(p, axis=-1, keepdims=True)
        p_scr[...] = p.astype(BF)

        def v_group(rg, c2):
            o_scr[...] = jnp.zeros((H, GW), F32)

            def v_unit(ch, c3):
                slot = advance(u0 + UPB + rg * NCH + ch)
                vt = buf[slot].reshape(GW, UC)
                col = pl.ds(pl.multiple_of(ch * UC, UC), UC)
                o_scr[...] += lax.dot_general(p_scr[:, col], vt, (((1,), (1,)), ((), ())),
                                              preferred_element_type=F32)
                return c3

            lax.fori_loop(0, NCH, v_unit, 0)

            @pl.when(jnp.logical_and(b == 0, rg == 0))
            def _():
                wait_all(wo_v, msem.at[3])

            ob = jnp.where(_head_mask(rg * GW, GW), o_scr[...] / l_scr[...], 0.0).astype(BF)
            wo_g = wo_v[pl.ds(pl.multiple_of(rg * GW, GW), GW), :]
            contrib = jnp.sum(jnp.dot(ob, wo_g, preferred_element_type=F32), axis=0, keepdims=True)
            rows = lax.broadcasted_iota(jnp.int32, (R, D), 0)
            acc_scr[...] += jnp.where(rows == b, contrib, 0.0)
            return c2

        lax.fori_loop(0, NRG, v_group, 0)
        return carry

    lax.fori_loop(0, B, batch, 0)

    hres = x8_scr[...] + acc_scr[...]
    hn = _layernorm(hres)
    hb = hn.astype(BF)
    wr_copy.wait()
    wr = wr_v[...].astype(F32)
    racc = hn[:, 0:128] * wr[0:1, :]
    for j in range(1, D // 128):
        racc = racc + hn[:, j * 128:(j + 1) * 128] * wr[j:j + 1, :]
    gate = jax.nn.sigmoid(jnp.sum(racc, axis=-1, keepdims=True))
    base = hres + hn + hn * 0.0

    wait_all(wg_v, msem.at[4])
    g = jnp.dot(hb, wg_v[...], preferred_element_type=F32)
    g = g * jax.nn.sigmoid(g)
    wait_all(wu_v, msem.at[5])
    u = jnp.dot(hb, wu_v[...], preferred_element_type=F32)
    act = (g * u).astype(BF)
    y = None
    for c in range(len(WD_GROUPS)):
        rows_c = pl.ds(WD_OFF[c], WD_GROUPS[c])
        wait_all(wd_v.at[rows_c], dsem.at[c])
        part = jnp.dot(act[:, WD_OFF[c]:WD_OFF[c] + WD_GROUPS[c]], wd_v[rows_c, :],
                       preferred_element_type=F32)
        y = part if y is None else y + part
    res = base + y * gate
    out_ref[...] = res[0:B, :].astype(BF)


@jax.jit
def pallas_sequential_preLN__mha_block_cached__moe_arch_mod__decode_kernel(
    A_x, A_k_cache, A_v_cache, A_wq, A_wo, B_x, B_w_r, B_w_gate, B_w_up, B_w_down,
):
    x2 = A_x.reshape(B, D)
    kt = jnp.swapaxes(A_k_cache, 2, 3).reshape(B * NRG, NA, NJ, 8, SK)
    vt = jnp.swapaxes(A_v_cache, 2, 3).reshape(B * NRG, NA, NJ, 8, SK)
    wr2 = B_w_r.reshape(D // 128, 128)
    any_spec = pl.BlockSpec(memory_space=pl.ANY)
    out = pl.pallas_call(
        _kernel,
        out_shape=jax.ShapeDtypeStruct((B, D), BF),
        in_specs=[any_spec] * 9,
        out_specs=pl.BlockSpec(memory_space=pltpu.VMEM),
        scratch_shapes=[
            pltpu.VMEM((B, D), BF),
            pltpu.VMEM((D // 128, 128), BF),
            pltpu.VMEM((D, HD), BF),
            pltpu.VMEM((HD, D), BF),
            pltpu.VMEM((D, F), BF),
            pltpu.VMEM((D, F), BF),
            pltpu.VMEM((F, D), BF),
            pltpu.VMEM((NSLOT, NA, NJ, 8, UC), BF),
            pltpu.VMEM((R, D), F32),
            pltpu.VMEM((B * NRG, H, GW), BF),
            pltpu.VMEM((H, SK), F32),
            pltpu.VMEM((H, SK), BF),
            pltpu.VMEM((H, 1), F32),
            pltpu.VMEM((H, GW), F32),
            pltpu.VMEM((R, D), F32),
            pltpu.SemaphoreType.DMA((NSLOT,)),
            pltpu.SemaphoreType.DMA((6,)),
            pltpu.SemaphoreType.DMA((len(WD_GROUPS),)),
        ],
        compiler_params=pltpu.CompilerParams(vmem_limit_bytes=100 * 1024 * 1024),
    )(x2, kt, vt, A_wq, A_wo, wr2, B_w_gate, B_w_up, B_w_down)
    return out.reshape(B, 1, D)
```
